```python
import os as _os
_os.environ.setdefault("JAX_PLATFORMS", "cpu")
import jax
import jax.numpy as jnp

def _softmax(x, axis=-1):
    return jax.nn.softmax(x, axis=axis)
def _gelu(x):
    return jax.nn.gelu(x, approximate=True)
def _silu(x):
    return jax.nn.silu(x)
def _sigmoid(x):
    return jax.nn.sigmoid(x)
def _layernorm(x, axis=-1, eps=1e-5):
    m = jnp.mean(x, axis=axis, keepdims=True)
    v = jnp.var(x, axis=axis, keepdims=True)
    return (x - m) / jnp.sqrt(v + eps)
def _scatter_add(tgt, idx, src, axis=0):
    return tgt.at[idx].add(src)
def _segment_sum(src, seg, n):
    return jax.ops.segment_sum(src, seg, n)
class _Rng:
    def __init__(self, key):
        self._k = key
    def _next(self):
        self._k, sub = jax.random.split(self._k)
        return sub
    def normal(self, shape):
        return jax.random.normal(self._next(), shape, dtype=jnp.bfloat16)
    def randint(self, lo, hi, shape):
        return jax.random.randint(self._next(), shape, lo, hi, dtype=jnp.int32)
    def uniform(self, shape, lo=0.0, hi=1.0):
        return jax.random.uniform(self._next(), shape, jnp.bfloat16, lo, hi)
    def permutation(self, n):
        return jax.random.permutation(self._next(), n)


kernel_name = 'concat_heads__mha_block_cached__gqa_block_cached__near_ridge'

def setup_inputs():
    _rng = _Rng(jax.random.key(int.from_bytes(__import__("os").urandom(4), "little")))
    _w = (lambda a: (lambda t: t.astype(jnp.bfloat16) if jnp.issubdtype(t.dtype, jnp.floating) else t)(jnp.asarray(a)))
    def _A_setup():
        B, Sq, D = 8, 128, 512
        H, Sk, Dh = 32, 1024, 128
        return {
            "x": _w((lambda *s: _rng.normal(s) * 0.8)(B, Sq, D)),
            "k_cache": _w((lambda *s: _rng.normal(s) * 0.8)(B, H, Sk, Dh)),
            "v_cache": _w((lambda *s: _rng.normal(s) * 0.05)(B, H, Sk, Dh)),
            "wq": _w((lambda *s: _rng.normal(s) * 0.8)(D, H * Dh) * (D ** -0.5)),
            "wo": _w((lambda *s: _rng.normal(s) * 0.05)(H * Dh, D) * ((H * Dh) ** -0.5)),
        }
    _A_in = _A_setup()

    def _B_setup():
        B, Sq, D = 8, 128, 512
        Hq, Hkv, Sk, Dh = 32, 32, 1024, 128
        assert Hq % Hkv == 0, (Hq, Hkv)
        return {
            "x": _w((lambda *s: _rng.normal(s) * 0.8)(B, Sq, D)),
            "k_cache": _w((lambda *s: _rng.normal(s) * 0.8)(B, Hkv, Sk, Dh)),
            "v_cache": _w((lambda *s: _rng.normal(s) * 0.05)(B, Hkv, Sk, Dh)),
            "wq": _w((lambda *s: _rng.normal(s) * 0.8)(D, Hq * Dh) * (D ** -0.5)),
            "wo": _w((lambda *s: _rng.normal(s) * 0.05)(Hq * Dh, D) * ((Hq * Dh) ** -0.5)),
        }
    _B_in = _B_setup()

    return {
        "A_x": _A_in["x"],
        "A_k_cache": _A_in["k_cache"],
        "A_v_cache": _A_in["v_cache"],
        "A_wq": _A_in["wq"],
        "A_wo": _A_in["wo"],
        "B_x": _B_in["x"],
        "B_k_cache": _B_in["k_cache"],
        "B_v_cache": _B_in["v_cache"],
        "B_wq": _B_in["wq"],
        "B_wo": _B_in["wo"],
    }

def reference(A_x, A_k_cache, A_v_cache, A_wq, A_wo, B_x, B_k_cache, B_v_cache, B_wq, B_wo):
    def _A_ref(x, k_cache, v_cache, wq, wo):
        B, Sq, D = x.shape
        H, Dh = 32, 128
        q = (lambda x, *d: x.transpose(*d))((x @ wq).reshape(B, Sq, H, Dh), 0, 2, 1, 3)
        scores = jnp.einsum("bhqd,bhkd->bhqk", q, k_cache) * (Dh ** -0.5)
        p = _softmax(scores, axis=-1)
        o = jnp.einsum("bhqk,bhkd->bhqd", p, v_cache)
        return (lambda x, *d: x.transpose(*d))(o, 0, 2, 1, 3).reshape(B, Sq, H * Dh) @ wo

    def _B_ref(x, k_cache, v_cache, wq, wo):
        B, Sq, D = x.shape
        Hq, Dh = 32, 128
        Hkv = k_cache.shape[1]
        rep = Hq // Hkv
        q = (lambda x, *d: x.transpose(*d))((x @ wq).reshape(B, Sq, Hq, Dh), 0, 2, 1, 3)
        k = jnp.repeat(k_cache, rep, axis=1)
        v = jnp.repeat(v_cache, rep, axis=1)
        scores = jnp.einsum("bhqd,bhkd->bhqk", q, k) * (Dh ** -0.5)
        p = _softmax(scores, axis=-1)
        o = jnp.einsum("bhqk,bhkd->bhqd", p, v)
        return (lambda x, *d: x.transpose(*d))(o, 0, 2, 1, 3).reshape(B, Sq, Hq * Dh) @ wo

    a = _A_ref(A_x, A_k_cache, A_v_cache, A_wq, A_wo)
    b = _B_ref(B_x, B_k_cache, B_v_cache, B_wq, B_wo)
    return jnp.concatenate([a, b], axis=-1)
```

```python
import jax
import jax.numpy as jnp
import jax.experimental.pallas as pl
import jax.experimental.pallas.tpu as pltpu

HG = 4
NBUF = 4
NB, NH, SQ, D, SK, DH = 8, 32, 128, 512, 1024, 128
G = NH // HG
W = HG * DH
LG = G.bit_length() - 1
SCALE = DH ** -0.5 * 1.4426950408889634


def _kernel(ax, ak, av, awq, awo, bx, bk, bv, bwq, bwo, out_hbm,
            kbuf, vbuf, xbuf, wqbuf, wobuf, acc, obuf, qsc, osc, sems, xsem, osem):
    n = NB * 2 * G
    srcs = ((ak, av, awq, awo), (bk, bv, bwq, bwo))

    def idx(i):
        i = jnp.asarray(i, jnp.int32)
        return i >> (LG + 1), (i >> LG) & 1, i & (G - 1)

    def copies(i, br_static, with_w):
        b, br, g = idx(i)
        slot = jax.lax.rem(jnp.asarray(i, jnp.int32), NBUF)
        k, v, wq, wo = srcs[br_static]
        off = pl.multiple_of(g * W, W)
        if with_w:
            return [
                pltpu.make_async_copy(wq.at[:, pl.ds(off, W)], wqbuf.at[br, g], sems.at[slot, 2]),
                pltpu.make_async_copy(wo.at[pl.ds(off, W), :], wobuf.at[br, g], sems.at[slot, 3]),
            ]
        return [
            pltpu.make_async_copy(k.at[b, pl.ds(g * HG, HG)], kbuf.at[slot], sems.at[slot, 0]),
            pltpu.make_async_copy(v.at[b, pl.ds(g * HG, HG)], vbuf.at[slot], sems.at[slot, 1]),
        ]

    def start(i):
        b, br, g = idx(i)
        for s in range(2):
            @pl.when(br == s)
            def _():
                @pl.when(b == 0)
                def _():
                    for c in copies(i, s, True):
                        c.start()
                for c in copies(i, s, False):
                    c.start()

    def wait_w(i):
        @pl.when(jnp.asarray(i, jnp.int32) < 2 * G)
        def _():
            for c in copies(i, 0, True):
                c.wait()

    def wait_kv(i):
        for c in copies(i, 0, False):
            c.wait()

    def ocopy(b, br):
        return pltpu.make_async_copy(
            obuf, out_hbm.at[b, :, pl.ds(pl.multiple_of(br * D, D), D)], osem.at[0])

    xc = [pltpu.make_async_copy(ax, xbuf.at[0], xsem.at[0]),
          pltpu.make_async_copy(bx, xbuf.at[1], xsem.at[1])]
    xc[0].start()
    start(0)
    xc[1].start()
    for i in range(1, NBUF - 1):
        start(i)
    xc[0].wait()
    xc[1].wait()

    def qproj(i):
        b, br, g = idx(i)
        q = jnp.dot(xbuf[br, b], wqbuf[br, g], preferred_element_type=jnp.float32)
        return (q * SCALE).astype(jnp.bfloat16)

    def oproj(i):
        b, br, g = idx(i)
        r = jnp.dot(osc[...], wobuf[br, g], preferred_element_type=jnp.float32)
        acc[...] = jnp.where(g == 0, r, acc[...] + r)

    def flush(i):
        b, br, g = idx(i)

        @pl.when(g == G - 1)
        def _():
            @pl.when(i >= G)
            def _():
                ocopy(0, 0).wait()
            obuf[...] = acc[...].astype(obuf.dtype)
            ocopy(b, br).start()

    wait_w(0)
    qsc[...] = qproj(0)
    osc[...] = jnp.zeros_like(osc)
    acc[...] = jnp.zeros_like(acc)

    def body(i, _):
        slot = jax.lax.rem(i, NBUF)

        @pl.when(i + NBUF - 1 < n)
        def _():
            start(i + NBUF - 1)
        wait_kv(i)
        wait_w(i + 1)

        ip = jnp.maximum(i - 1, 0)
        q = qsc[...]
        oproj(ip)
        os_ = []
        for h in range(HG):
            s = jax.lax.dot_general(q[:, h * DH:(h + 1) * DH], kbuf[slot, h], (((1,), (1,)), ((), ())),
                                    preferred_element_type=jnp.float32)
            m = jnp.max(s, axis=-1, keepdims=True)
            p = jnp.exp2(s - m)
            l = jnp.sum(p, axis=-1, keepdims=True)
            o = jnp.dot(p.astype(jnp.bfloat16), vbuf[slot, h], preferred_element_type=jnp.float32)
            osc[:, h * DH:(h + 1) * DH] = (o * (1.0 / l)).astype(jnp.bfloat16)
        qsc[...] = qproj(jnp.minimum(i + 1, n - 1))

        @pl.when(i > 0)
        def _():
            flush(ip)

    jax.lax.fori_loop(0, n, body, None)
    oproj(n - 1)
    flush(jnp.int32(n - 1))
    ocopy(0, 0).wait()


@jax.jit
def pallas_concat_heads__mha_block_cached__gqa_block_cached__near_ridge_kernel(
    A_x, A_k_cache, A_v_cache, A_wq, A_wo, B_x, B_k_cache, B_v_cache, B_wq, B_wo):
    a = pl.BlockSpec(memory_space=pl.ANY)
    bf = jnp.bfloat16
    return pl.pallas_call(
        _kernel,
        in_specs=[a] * 10,
        out_specs=a,
        out_shape=jax.ShapeDtypeStruct((NB, SQ, 2 * D), bf),
        scratch_shapes=[
            pltpu.VMEM((NBUF, HG, SK, DH), bf), pltpu.VMEM((NBUF, HG, SK, DH), bf),
            pltpu.VMEM((2, NB, SQ, D), bf),
            pltpu.VMEM((2, G, D, W), bf), pltpu.VMEM((2, G, W, D), bf),
            pltpu.VMEM((SQ, D), jnp.float32), pltpu.VMEM((SQ, D), bf),
            pltpu.VMEM((SQ, W), bf), pltpu.VMEM((SQ, W), bf),
            pltpu.SemaphoreType.DMA((NBUF, 4)), pltpu.SemaphoreType.DMA((2,)), pltpu.SemaphoreType.DMA((1,))],
        compiler_params=pltpu.CompilerParams(disable_bounds_checks=True, vmem_limit_bytes=100 * 1024 * 1024),
    )(A_x, A_k_cache, A_v_cache, A_wq, A_wo, B_x, B_k_cache, B_v_cache, B_wq, B_wo)
```
